```python
import os as _os
_os.environ.setdefault('JAX_PLATFORMS', 'cpu')
import jax
import jax.numpy as jnp

def _softmax(x, axis=-1):
    return jax.nn.softmax(x, axis=axis)

def _gelu(x):
    return jax.nn.gelu(x, approximate=True)

def _silu(x):
    return jax.nn.silu(x)

def _sigmoid(x):
    return jax.nn.sigmoid(x)

def _layernorm(x, axis=-1, eps=1e-05):
    m = jnp.mean(x, axis=axis, keepdims=True)
    v = jnp.var(x, axis=axis, keepdims=True)
    return (x - m) / jnp.sqrt(v + eps)

def _scatter_add(tgt, idx, src, axis=0):
    return tgt.at[idx].add(src)

def _segment_sum(src, seg, n):
    return jax.ops.segment_sum(src, seg, n)

class _Rng:

    def __init__(self, key):
        self._k = key

    def _next(self):
        self._k, sub = jax.random.split(self._k)
        return sub

    def normal(self, shape):
        return jax.random.normal(self._next(), shape, dtype=jnp.bfloat16)

    def randint(self, lo, hi, shape):
        return jax.random.randint(self._next(), shape, lo, hi, dtype=jnp.int32)

    def uniform(self, shape, lo=0.0, hi=1.0):
        return jax.random.uniform(self._next(), shape, jnp.bfloat16, lo, hi)

    def permutation(self, n):
        return jax.random.permutation(self._next(), n)
kernel_name = 'adaLN_cond__memory_aug_recurrent_mem_tr__moe_arch_mod__prompt'

def setup_inputs():
    _rng = _Rng(jax.random.key(int.from_bytes(__import__("os").urandom(4), "little")))
    _w = lambda a: (lambda t: t.astype(jnp.bfloat16) if jnp.issubdtype(t.dtype, jnp.floating) else t)(jnp.asarray(a))

    def _A_setup():
        B, S, Dm = (1, 2048, 448)
        H, Dh = (16, 256)
        M, seg = (8, 32)
        seg = min(seg, S)
        S = S // seg * seg
        return {'x': _w((lambda *s: _rng.normal(s) * 0.05)(B, S, Dm)), 'mem0': _w((lambda *s: _rng.normal(s) * 0.4)(B, M, Dm)), 'Wq': _w((lambda *s: _rng.normal(s) * 1.6)(Dm, H, Dh) * Dm ** (-0.5)), 'Wk': _w((lambda *s: _rng.normal(s) * 1.6)(Dm, H, Dh) * Dm ** (-0.5)), 'Wv': _w((lambda *s: _rng.normal(s) * 0.4)(Dm, H, Dh) * Dm ** (-0.5)), 'Wo': _w((lambda *s: _rng.normal(s) * 0.4)(H, Dh, Dm) * (H * Dh) ** (-0.5)), 'seg_len': seg}
    _A_in = _A_setup()

    def _B_setup():
        B, S, D, F, C = (1, 2048, 448, 1792, 1)
        return {'x': _w((lambda *s: _rng.normal(s) * 0.05)(B, S, D)), 'w_r': _w((lambda *s: _rng.normal(s) * 0.05)(D)), 'w_gate': _w((lambda *s: _rng.normal(s) * 0.05)(D, F)), 'w_up': _w((lambda *s: _rng.normal(s) * 0.05)(D, F)), 'w_down': _w((lambda *s: _rng.normal(s) * 0.05)(F, D))}
    _B_in = _B_setup()
    return {'A_x': _A_in['x'], 'A_mem0': _A_in['mem0'], 'A_Wq': _A_in['Wq'], 'A_Wk': _A_in['Wk'], 'A_Wv': _A_in['Wv'], 'A_Wo': _A_in['Wo'], 'A_seg_len': _A_in['seg_len'], 'B_x': _B_in['x'], 'B_w_r': _B_in['w_r'], 'B_w_gate': _B_in['w_gate'], 'B_w_up': _B_in['w_up'], 'B_w_down': _B_in['w_down'], 'c': _w((lambda *s: _rng.normal(s) * 0.05)(1, 448) * 8.0), 'w_mod': _w((lambda *s: _rng.normal(s) * 0.05)(448, 6 * 448) * 448 ** (-0.5) * 8.0)}

def reference(A_x, A_mem0, A_Wq, A_Wk, A_Wv, A_Wo, A_seg_len, B_x, B_w_r, B_w_gate, B_w_up, B_w_down, c, w_mod):

    def _A_ref(x, mem0, Wq, Wk, Wv, Wo, seg_len):
        B, S, Dm = x.shape
        H, Dh = (Wq.shape[1], Wq.shape[2])
        M = mem0.shape[1]
        scale = Dh ** (-0.5)
        n_seg = S // seg_len
        L = M + seg_len
        idx = jnp.arange(L)
        mask = (idx[:, None] < M) | (idx[:, None] >= idx[None, :])
        mem = mem0
        outs = []
        for s in range(n_seg):
            xs = x[:, s * seg_len:(s + 1) * seg_len, :].copy()
            h = jnp.concatenate([mem, xs], axis=1)
            q = jnp.einsum('btd,dhe->bhte', h, Wq)
            k = jnp.einsum('btd,dhe->bhte', h, Wk)
            v = jnp.einsum('btd,dhe->bhte', h, Wv)
            scores = jnp.einsum('bhqe,bhke->bhqk', q, k) * scale
            scores = jnp.where(mask[None, None], scores, -1000000000.0)
            p = _softmax(scores, axis=-1)
            o = jnp.einsum('bhqk,bhke->bhqe', p, v)
            o = jnp.einsum('bhte,hed->btd', o, Wo)
            mem = o[:, :M, :].copy()
            outs.append(o[:, M:, :])
        return jnp.concatenate(outs, axis=1)

    def _B_ref(x, w_r, w_gate, w_up, w_down):
        B, S, D = x.shape
        C = 1
        r = x @ w_r
        idx = jnp.argsort(-r, axis=-1)[:, :C]
        idx_e = jnp.repeat(idx.reshape(B, C, 1), D, axis=2)
        x_sel = jnp.take_along_axis(x, idx_e, axis=1)
        g = _silu(x_sel @ w_gate)
        u = x_sel @ w_up
        y = g * u @ w_down
        r_sel = _sigmoid(jnp.take_along_axis(r, idx, axis=1))
        y = y * r_sel.reshape(B, C, 1)
        b_off = (jnp.arange(B) * S).reshape(B, 1)
        flat_idx = (idx + b_off).reshape(B * C)
        zero = (x * 0.0).reshape(B * S, D)
        upd = _scatter_add(zero, flat_idx, y.reshape(B * C, D), axis=0)
        return x + upd.reshape(B, S, D)
    x = A_x
    mod = (_silu(c) @ w_mod).reshape(c.shape[0], 6, 1, -1)
    sa, ca, ga, sb, cb, gb = (mod[:, 0].copy(), mod[:, 1].copy(), mod[:, 2].copy(), mod[:, 3].copy(), mod[:, 4].copy(), mod[:, 5].copy())
    h = _layernorm(x, axis=-1) * (1 + ca) + sa
    x = x + ga * _A_ref(h, A_mem0, A_Wq, A_Wk, A_Wv, A_Wo, A_seg_len)
    h = _layernorm(x, axis=-1) * (1 + cb) + sb
    x = x + gb * _B_ref(h, B_w_r, B_w_gate, B_w_up, B_w_down)
    return x
```

```python
import functools

import jax
import jax.numpy as jnp
from jax import lax
import jax.experimental.pallas as pl
import jax.experimental.pallas.tpu as pltpu

F32 = jnp.float32
BF16 = jnp.bfloat16
U32 = jnp.uint32

S, D, H, E, M, SEG, FF = 2048, 448, 16, 256, 8, 32, 1792
NSEG = S // SEG
DM = 384
DH = D - DM
DX = 512
NT = 56
EPS = 1e-5
TB = 128
NB = S // TB
DC = 64
NC = D // DC
TIE = True


def _r(x):
    return x.astype(BF16).astype(F32)


def _dot(a, b):
    return jnp.dot(a, b, preferred_element_type=F32)


def _dot_t(a, b):
    return lax.dot_general(a, b, (((1,), (1,)), ((), ())), preferred_element_type=F32)


def _pack(x):
    return pltpu.bitcast(x.astype(BF16), U32)


def _unpack(x):
    return pltpu.bitcast(x, BF16)


def _fold8(v):
    return jnp.sum(v.reshape(v.shape[0] // 8, 8, v.shape[1]), axis=0)


def _group8_reduce(v, op, lane):
    for d in (1, 2, 4):
        a = pltpu.roll(v, d, 1)
        b = pltpu.roll(v, 128 - d, 1)
        v = op(v, jnp.where((lane & d) != 0, a, b))
    return v


FT = [(0, 128), (128, 128), (256, 128), (384, 64)]


def _kernel(xt_hbm, mem0_ref, wq_hbm, wk_hbm, wv_hbm, wot_hbm, wr_ref, wg_hbm, wu_hbm, wdt_hbm,
            c_ref, wmod_hbm, o_ref,
            xt_ref, wraw_ref, wot_ref, wg_ref, wu_ref, wdt_ref, wmod_ref,
            h_ref, a_ref, wt_ref, wK_ref, wV_ref, stK_ref, stV_ref, col_ref, r_ref, x1_ref, z_ref,
            sems):
    def w_copy(wi, cidx):
        src = (wq_hbm, wk_hbm, wv_hbm)[wi]
        return pltpu.make_async_copy(src.at[pl.ds(cidx * DC, DC)],
                                     wraw_ref.at[wi, pl.ds(cidx * DC, DC)], sems.at[wi * NC + cidx])

    def o_copy(p):
        return pltpu.make_async_copy(wot_hbm.at[pl.ds(2 * p, 2)], wot_ref.at[pl.ds(2 * p, 2)],
                                     sems.at[3 * NC + p])

    x_copy = pltpu.make_async_copy(xt_hbm.at[0], xt_ref, sems.at[3 * NC + 8])
    mod_copy = pltpu.make_async_copy(wmod_hbm, wmod_ref, sems.at[3 * NC + 9])
    mlp_copies = [pltpu.make_async_copy(s_, d_, sems.at[3 * NC + 10 + i]) for i, (s_, d_) in
                  enumerate(((wg_hbm, wg_ref), (wu_hbm, wu_ref), (wdt_hbm, wdt_ref)))]

    for cidx in range(NC):
        w_copy(2, cidx).start()
    for p in range(H // 2):
        o_copy(p).start()
    for wi in (0, 1):
        for cidx in range(NC):
            w_copy(wi, cidx).start()
    mod_copy.start()
    x_copy.start()
    for cp in mlp_copies:
        cp.start()

    z_ref[...] = jnp.zeros((8, 128), U32)
    a_ref[0:TB // 2, :] = jnp.zeros((TB // 2, DX), U32)

    def swap(wi, cidx):
        w_copy(wi, cidx).wait()
        v = jnp.swapaxes(wraw_ref[wi, cidx * DC:(cidx + 1) * DC], 0, 1)
        wt_ref[wi, :, cidx * DC // 2:(cidx + 1) * DC // 2, :] = pltpu.bitcast(v, U32)

    def fold_store(p, mats, w_ref):
        for t in range(2):
            hh = 2 * p + t
            for j in range(3):
                col = pl.multiple_of((j * H + hh) * 128, 128)
                w_ref[:, pl.ds(col, 128)] = _pack(mats[t][:, j * 128:(j + 1) * 128])
        col = pl.multiple_of((3 * H + p) * 128, 128)
        w_ref[:, pl.ds(col, 128)] = _pack(jnp.concatenate([m_[:, DM:] for m_ in mats], axis=1))

    for cidx in range(NC):
        swap(2, cidx)

    def fold_v(p, carry):
        o_copy(p).wait()
        fold_store(p, [_dot_t(_unpack(wt_ref[2, 2 * p + t]), wot_ref[2 * p + t]) for t in range(2)],
                   wV_ref)
        return carry
    lax.fori_loop(0, H // 2, fold_v, 0)

    for wi in (0, 1):
        for cidx in range(NC):
            swap(wi, cidx)

    def fold_k(p, carry):
        fold_store(p, [_dot_t(_unpack(wt_ref[1, 2 * p + t]), _unpack(wt_ref[0, 2 * p + t]))
                       * (E ** -0.5) for t in range(2)], wK_ref)
        return carry
    lax.fori_loop(0, H // 2, fold_k, 0)

    mod_copy.wait()
    cc = c_ref[...].astype(F32)
    sc = _r(cc * jax.nn.sigmoid(cc))
    sc8 = jnp.broadcast_to(sc, (8, D)).astype(BF16)
    mod = _r(_dot(sc8, wmod_ref[...]))[0:1]
    for i in range(6):
        v = mod[:, i * D:(i + 1) * D]
        if i in (1, 4):
            v = _r(1.0 + v)
        col_ref[i] = jnp.broadcast_to(v, (TB, D)).T
    col_ref[6] = jnp.broadcast_to(wr_ref[...].astype(F32), (TB, D)).T
    x_copy.wait()

    def stats_mean(acc):
        return jnp.sum(acc, axis=0, keepdims=True) * (1.0 / D)

    def stats_inv(acc):
        var = jnp.sum(acc, axis=0, keepdims=True) * (1.0 / D)
        return 1.0 / _r(jnp.sqrt(_r(_r(var) + EPS)))

    def ln1_pieces(b):
        t0 = pl.multiple_of(b * TB, TB)
        st = {}

        def load(k):
            f0, n = FT[k]
            return xt_ref[f0:f0 + n, pl.ds(t0, TB)].astype(F32)

        def p1(k):
            s_ = _fold8(load(k))
            st['s'] = s_ if k == 0 else st['s'] + s_
            return st['s']

        def p2(k):
            if k == 0:
                st['mean'] = stats_mean(st['s'])
            xc = load(k) - st['mean']
            s_ = _fold8(xc * xc)
            st['q'] = s_ if k == 0 else st['q'] + s_
            return st['q']

        def p3(k):
            if k == 0:
                st['inv'] = stats_inv(st['q'])
                st['m'] = _r(st['mean'])
            f0, n = FT[k]
            h = (load(k) - st['m']) * st['inv'] * col_ref[1, f0:f0 + n] + col_ref[0, f0:f0 + n]
            if n < 128:
                h = jnp.concatenate([h, h], axis=0)
            ht = h.T
            h_ref[pl.ds(t0, TB), 128 * k:128 * k + 128] = ht
            return _fold8(ht)

        return [functools.partial(f, k) for f in (p1, p2, p3) for k in range(4)]

    def post_pieces(b, final=None):
        t0 = pl.multiple_of(b * TB, TB)
        r0 = pl.multiple_of(b * (TB // 2), TB // 2)
        st = {}

        def p1(k):
            f0, n = FT[k]
            a = _unpack(a_ref[pl.ds(r0, TB // 2), 128 * k:128 * k + 128]).T[:n].astype(F32)
            x = xt_ref[f0:f0 + n, pl.ds(t0, TB)].astype(F32)
            x1 = _r(x + col_ref[2, f0:f0 + n] * a)
            x1_ref[f0:f0 + n, :] = x1
            s_ = _fold8(x1)
            st['s'] = s_ if k == 0 else st['s'] + s_
            return st['s']

        def p2(k):
            if k == 0:
                st['mean'] = stats_mean(st['s'])
            f0, n = FT[k]
            xc = x1_ref[f0:f0 + n, :] - st['mean']
            s_ = _fold8(xc * xc)
            st['q'] = s_ if k == 0 else st['q'] + s_
            return st['q']

        def p3(k):
            if k == 0:
                st['inv'] = stats_inv(st['q'])
                st['m'] = _r(st['mean'])
            f0, n = FT[k]
            x1 = x1_ref[f0:f0 + n, :]
            h2 = _r((x1 - st['m']) * st['inv'] * col_ref[4, f0:f0 + n] + col_ref[3, f0:f0 + n])
            s_ = _fold8(h2 * col_ref[6, f0:f0 + n])
            st['r'] = s_ if k == 0 else st['r'] + s_
            if final is None:
                o_ref[0, f0:f0 + n, pl.ds(t0, TB)] = (x1 + col_ref[5, f0:f0 + n] * h2).astype(BF16)
                if k == 3:
                    r_ref[pl.ds(b, 1), :] = _r(jnp.sum(st['r'], axis=0, keepdims=True))
            else:
                final.append(h2)
                if k == 3:
                    final.append(_r(jnp.sum(st['r'], axis=0, keepdims=True)))
            return st['r']

        return [functools.partial(f, k) for f in (p1, p2, p3) for k in range(4)]

    for pc in ln1_pieces(0):
        pc()

    lane8 = lax.broadcasted_iota(jnp.int32, (8, 128), 1)
    lo_half = lane8 < DH
    lane40 = lax.broadcasted_iota(jnp.int32, (M + SEG, 128), 1)
    row40 = lax.broadcasted_iota(jnp.int32, (M + SEG, 128), 0)

    def proj_chunk(lhs, w_ref, st_ref, j, c, dests, sched):
        c0 = (j * H + 4 * c) * 128
        piece = sched.pop(0) if sched else None
        if piece is None:
            w = w_ref[:, c0:c0 + 512]
        else:
            tok = pltpu.bitcast(piece(), U32)
            if TIE:
                w00 = w_ref[0:8, c0:c0 + 128] | (tok & z_ref[...])
                w = jnp.concatenate(
                    [jnp.concatenate([w00, w_ref[0:8, c0 + 128:c0 + 512]], axis=1),
                     w_ref[8:, c0:c0 + 512]], axis=0)
            else:
                w = w_ref[:, c0:c0 + 512]
        y = _dot(lhs, _unpack(w))
        for g, (bi, gi) in enumerate(dests):
            if j < 3:
                blk = jnp.concatenate(
                    [y[8 * g:8 * g + 8, 128 * t:128 * t + 128] for t in range(4)], axis=0)
                st_ref[bi, gi, 16 * c:16 * c + 16, 128 * j:128 * j + 128] = _pack(blk)
            else:
                pieces = []
                for t in range(4):
                    v = y[8 * g:8 * g + 8, 128 * t:128 * t + 128]
                    pieces.append(jnp.where(lo_half, v, 0.0))
                    pieces.append(jnp.where(lo_half, 0.0, v))
                blk = jnp.concatenate(pieces, axis=0)
                st_ref[bi, gi, 32 * c:32 * c + 32, DM:DX] = _pack(blk)

    chunks = [(3, 0), (3, 1)] + [(j, c) for j in range(3) for c in range(4)]

    def segment(bi, hq, lhs, dests, r0, sched):
        for (j, c) in chunks:
            proj_chunk(lhs, wK_ref, stK_ref, j, c, dests, sched)
        sc_g = []
        proj_chunk(lhs, wV_ref, stV_ref, *chunks[0], dests, sched)
        for g in (4, 0, 1, 2, 3):
            sg = _r(_dot_t(hq, _unpack(stK_ref[bi, g]))[:M + SEG])
            if g > 0:
                key = 8 * g + (lane40 & 7)
                sg = jnp.where((row40 < M) | (row40 >= key), sg, -1e9)
            sc_g.append(sg)
            if len(sc_g) in (2, 4):
                proj_chunk(lhs, wV_ref, stV_ref, *chunks[len(sc_g) // 2], dests, sched)
        sc_g = sc_g[1:] + sc_g[:1]
        mx = functools.reduce(jnp.maximum, sc_g)
        mx = _group8_reduce(mx, jnp.maximum, lane40)
        ex = [jnp.exp(sg - mx) for sg in sc_g]
        den = _group8_reduce(functools.reduce(jnp.add, ex), jnp.add, lane40)
        inv = 1.0 / den
        p = jnp.concatenate([e * inv for e in ex], axis=1)
        p = jnp.concatenate([p, jnp.zeros((8, 640), F32)], axis=0).astype(BF16)
        for (j, c) in chunks[3:]:
            proj_chunk(lhs, wV_ref, stV_ref, j, c, dests, sched)
        outs = {}
        for j in (3, 0, 1, 2):
            vj = _unpack(stV_ref[bi, :, :, 128 * j:128 * j + 128].reshape(320, 128))
            outs[j] = _dot(p, vj)[:M + SEG]
        hi = outs[3] + pltpu.roll(outs[3], DH, 1)
        o = jnp.concatenate([outs[0], outs[1], outs[2], hi], axis=1)
        a_ref[pl.ds(r0, SEG // 2), :] = _pack(o[M:])
        return _r(o[:M])

    def block(i, mem):
        pa = post_pieces(jnp.maximum(i - 1, 0))
        pb = ln1_pieces(jnp.minimum(i + 1, NB - 1))
        sched = []
        for u, v in zip(pa, pb):
            sched += [None, None, None, u, None, None, None, v]
        for half in range(2):
            r0 = pl.multiple_of(i * TB + half * 2 * SEG, 2 * SEG)
            ra = pl.multiple_of(i * (TB // 2) + half * SEG, SEG)
            ha = h_ref[pl.ds(r0, SEG), :]
            hb = h_ref[pl.ds(r0 + SEG, SEG), :]
            hq = jnp.concatenate([mem, ha, hb[24:]], axis=0).astype(BF16)
            mem = segment(0, hq, hq[:, :D], [(0, 0), (0, 1), (0, 2), (0, 3), (0, 4), (1, 4)],
                          ra, sched)
            hb = h_ref[pl.ds(r0 + SEG, SEG), :]
            hq = jnp.concatenate([mem, hb, jnp.zeros((8, DX), F32)], axis=0).astype(BF16)
            mem = segment(1, hq, hq[:32, :D], [(1, 0), (1, 1), (1, 2), (1, 3)],
                          ra + SEG // 2, sched)
        assert not any(sched)
        return mem

    m0 = mem0_ref[0].astype(F32)
    m0 = jnp.concatenate([m0, m0[:, DM:]], axis=1)
    lax.fori_loop(0, NB, block, m0)

    for pc in post_pieces(NB - 1):
        pc()

    for cp in mlp_copies:
        cp.wait()
    rall = r_ref[...]
    tok = (lax.broadcasted_iota(jnp.int32, (NB, TB), 0) * TB
           + lax.broadcasted_iota(jnp.int32, (NB, TB), 1))
    top = jnp.max(rall)
    idx = jnp.min(jnp.where(rall == top, tok, S))
    idx = jnp.clip(idx, 0, S - 1)
    blk = idx // TB
    ln = idx - blk * TB
    fin = []
    for pc in post_pieces(blk, fin):
        pc()
    h2 = jnp.concatenate(fin[:4], axis=0)
    r = fin[4]
    t0 = pl.multiple_of(blk * TB, TB)
    onehot = (lax.broadcasted_iota(jnp.int32, (8, TB), 1) == ln)
    hsel = _dot_t(onehot.astype(BF16), h2.astype(BF16)).astype(BF16)
    gt = _r(_dot(hsel, wg_ref[...]))
    gt = _r(gt * jax.nn.sigmoid(gt))
    up = _r(_dot(hsel, wu_ref[...]))
    act = jnp.broadcast_to(_r(gt * up)[0:1], (TB, FF)).astype(BF16)
    yt = _r(_dot_t(wdt_ref[...], act))
    yt = _r(yt * _r(jax.nn.sigmoid(r)))
    sel = lax.broadcasted_iota(jnp.int32, (D, TB), 1) == ln
    hb2 = jnp.where(sel, _r(h2 + yt), h2)
    o_ref[0, :, pl.ds(t0, TB)] = (x1_ref[...] + col_ref[5] * hb2).astype(BF16)


@functools.partial(jax.jit, static_argnames=("A_seg_len",))
def pallas_adaLN_cond__memory_aug_recurrent_mem_tr__moe_arch_mod__prompt_kernel(A_x, A_mem0, A_Wq, A_Wk, A_Wv, A_Wo, A_seg_len, B_x, B_w_r, B_w_gate, B_w_up,
              B_w_down, c, w_mod):
    assert A_seg_len == SEG
    any_spec = pl.BlockSpec(memory_space=pl.ANY)
    vmem_spec = pl.BlockSpec(memory_space=pltpu.VMEM)
    out_t = pl.pallas_call(
        _kernel,
        out_shape=jax.ShapeDtypeStruct((1, D, S), BF16),
        in_specs=[any_spec, vmem_spec, any_spec, any_spec, any_spec, any_spec, vmem_spec,
                  any_spec, any_spec, any_spec, vmem_spec, any_spec],
        out_specs=vmem_spec,
        scratch_shapes=[
            pltpu.VMEM((D, S), BF16),
            pltpu.VMEM((3, D, H, E), BF16),
            pltpu.VMEM((H, D, E), BF16),
            pltpu.VMEM((D, FF), BF16),
            pltpu.VMEM((D, FF), BF16),
            pltpu.VMEM((D, FF), BF16),
            pltpu.VMEM((D, 6 * D), BF16),
            pltpu.VMEM((S, DX), F32),
            pltpu.VMEM((S // 2, DX), U32),
            pltpu.VMEM((3, H, D // 2, E), U32),
            pltpu.VMEM((D // 2, NT * 128), U32),
            pltpu.VMEM((D // 2, NT * 128), U32),
            pltpu.VMEM((2, 5, 64, DX), U32),
            pltpu.VMEM((2, 5, 64, DX), U32),
            pltpu.VMEM((7, D, TB), F32),
            pltpu.VMEM((NB, TB), F32),
            pltpu.VMEM((D, TB), F32),
            pltpu.VMEM((8, 128), U32),
            pltpu.SemaphoreType.DMA((3 * NC + 13,)),
        ],
        compiler_params=pltpu.CompilerParams(vmem_limit_bytes=110 * 1024 * 1024),
    )(jnp.swapaxes(A_x, 1, 2), A_mem0, A_Wq, A_Wk, A_Wv, jnp.swapaxes(A_Wo, 1, 2),
      B_w_r.reshape(1, D), B_w_gate, B_w_up, B_w_down.T, c, w_mod)
    return jnp.swapaxes(out_t, 1, 2)
```

```python
import contextlib
import functools

import jax
import jax.numpy as jnp
from jax import lax
import jax.experimental.pallas as pl
import jax.experimental.pallas.tpu as pltpu

F32 = jnp.float32
BF16 = jnp.bfloat16
U32 = jnp.uint32

S, D, H, E, M, SEG, FF = 2048, 448, 16, 256, 8, 32, 1792
DM = 384
DH = D - DM
DX = 512
NT = 56
EPS = 1e-5
TB = 128
NB = S // TB
SCOPES = False
NFILL = (0, 1, 1, 1, 2)

POS = (None, 24, 8, 16, 0)
VIS = frozenset((q, g) for q in range(5) for g in range(5)
                if q == 0 or g == 0 or POS[q] >= POS[g])
QROWS = [1 + max(q // 2 for q in range(5) if (q, g) in VIS) for g in range(5)]
FT = [(0, 128), (128, 128), (256, 128), (384, 64)]
MODA = 2 * D


def _scope(name):
    return jax.named_scope(name) if SCOPES else contextlib.nullcontext()


def _r(x):
    return x.astype(BF16).astype(F32)


def _dot(a, b):
    return jnp.dot(a, b, preferred_element_type=F32)


def _dot_t(a, b):
    return lax.dot_general(a, b, (((1,), (1,)), ((), ())), preferred_element_type=F32)


def _pack(x):
    return pltpu.bitcast(x.astype(BF16), U32)


def _unpack(x):
    return pltpu.bitcast(x, BF16)


def _fold8(v):
    return jnp.sum(v.reshape(v.shape[0] // 8, 8, v.shape[1]), axis=0)


def _or8(v):
    return functools.reduce(jnp.bitwise_or, [v[8 * i:8 * i + 8] for i in range(v.shape[0] // 8)])


def _roll(v, s):
    s = s % 128
    return pltpu.roll(v, s, 1) if s else v


def _group8_reduce(v, op, lane):
    for d in (1, 2, 4):
        v = op(v, jnp.where((lane & d) != 0, _roll(v, d), _roll(v, -d)))
    return v


def _kernel(xt_hbm, mem0_ref, wq_hbm, wk_hbm, wv_hbm, wot_hbm, wr_ref, wg_hbm, wu_hbm, wdt_hbm,
            c_ref, wmod_hbm, o_hbm,
            xt_ref, rq_ref, rk_ref, rv_ref, wot_ref, wg_ref, wu_ref, wdt_ref, wmod_ref, ot_ref,
            h_ref, a_ref, tq_ref, tk_ref, tv_ref, wK_ref, wV_ref, st_ref, xc_ref, xn_ref,
            hr_ref, tt_ref, wG_ref, g_ref, gc_ref, gn_ref, zd_ref, od_ref, mod_ref, col_ref,
            r_ref, x1_ref, h2_ref, z_ref, sems):
    nsem = [0]

    def copy(src, dst):
        nsem[0] += 1
        return pltpu.make_async_copy(src, dst, sems.at[nsem[0] - 1])

    def rows_copy(src, dst, r0, n):
        return copy(src.at[pl.ds(r0, n)], dst.at[pl.ds(r0, n)])

    def cols_copy(src, dst, c0, n):
        return copy(src.at[:, pl.ds(c0, n)], dst.at[:, pl.ds(c0, n)])

    o_cp = [rows_copy(wot_hbm, wot_ref, a, b - a) for a, b in ((0, 8), (8, 12), (12, 16))]
    v_cp = [rows_copy(wv_hbm, rv_ref, 64 * i, 64) for i in range(7)]
    q_cp = [rows_copy(wq_hbm, rq_ref, f0, n) for f0, n in FT]
    k_cp = [rows_copy(wk_hbm, rk_ref, f0, n) for f0, n in FT]
    mod_cp = [cols_copy(wmod_hbm, wmod_ref, 0, MODA),
              cols_copy(wmod_hbm, wmod_ref, MODA, 6 * D - MODA)]
    x_cp = [cols_copy(xt_hbm.at[0], xt_ref, 0, 2 * TB),
            cols_copy(xt_hbm.at[0], xt_ref, 2 * TB, S - 2 * TB)]
    mlp_cp = [copy(wg_hbm, wg_ref), copy(wu_hbm, wu_ref), copy(wdt_hbm, wdt_ref)]
    for cp in ([o_cp[0]] + v_cp + o_cp[1:]
               + [q_cp[0], k_cp[0], k_cp[1], q_cp[1], q_cp[3], k_cp[2], q_cp[2], k_cp[3]]
               + [x_cp[0], mod_cp[0], mod_cp[1], x_cp[1]]):
        cp.start()

    z_ref[...] = jnp.zeros((8, 128), U32)
    a_ref[0:TB // 2, :] = jnp.zeros((TB // 2, DX), U32)
    tt_ref[:, :, DM:DX] = jnp.zeros((2, 32 * H, 128), U32)
    zd_ref[...] = jnp.zeros(zd_ref.shape, F32)
    od_ref[...] = jnp.zeros(od_ref.shape, F32)

    lane8 = lax.broadcasted_iota(jnp.int32, (8, 128), 1)
    lo_half = lane8 < DH
    lo32 = lax.broadcasted_iota(jnp.int32, (32, 128), 1) < DH
    w_refs = (wK_ref, wV_ref)
    l_refs = (tk_ref, tv_ref)
    scales = (E ** -0.5, 1.0)

    def tie(w, tok):
        if tok is None:
            return w
        w00 = w[0:8, 0:128] | (pltpu.bitcast(tok, U32) & z_ref[...])
        top = jnp.concatenate([w00, w[0:8, 128:]], axis=1)
        return jnp.concatenate([top, w[8:]], axis=0) if w.shape[0] > 8 else top

    def tie_rows(w, pcs):
        if not pcs:
            return w
        ng = w.shape[0] // 8
        slots = {}
        for k, pc in enumerate(pcs):
            slots.setdefault((k * ng) // len(pcs) * 8, []).append(pc)
        cuts = sorted(slots) + [ng * 8]
        out = []
        for a, b in zip(cuts[:-1], cuts[1:]):
            tok = functools.reduce(jnp.bitwise_or, [pltpu.bitcast(pc(), U32) for pc in slots[a]])
            out.append(tie(w[a:b], tok))
        return jnp.concatenate(out, axis=0)

    def region(units, pieces=(), skip=200):
        total = sum(c for c, _ in units)
        pieces = list(pieces)
        n, t, done = len(pieces), 0, 0
        for cost, fn in units:
            t += cost
            upto = n if t == total else max(0, (n * (t - skip)) // (total - skip))
            fn(pieces[done:upto])
            done = max(done, upto)

    def swap(raw_ref, t_ref, r0, n):
        v = pltpu.bitcast(jnp.swapaxes(raw_ref[r0:r0 + n], 0, 1), U32)
        t_ref[:, r0 // 2:(r0 + n) // 2, :] = v

    def swap_small(raw_ref, t_ref, r0, h0, c0):
        v = pltpu.bitcast(jnp.swapaxes(raw_ref[r0:r0 + 16, h0:h0 + 8, c0:c0 + 128], 0, 1), U32)
        t_ref[h0:h0 + 8, r0 // 2:r0 // 2 + 8, c0:c0 + 128] = v
        return functools.reduce(jnp.bitwise_or, [v[i] for i in range(8)])

    def swap_pieces(raw_ref, t_ref, r0, n):
        return [functools.partial(swap_small, raw_ref, t_ref, r, h0, c0)
                for r in range(r0, r0 + n, 16) for h0 in (0, 8) for c0 in (0, 128)]

    def r_rows(kv, hh, c0, c1):
        if kv == 0:
            return tq_ref[hh, c0 // 2:c1 // 2, :]
        return pltpu.bitcast(wot_ref[hh, c0:c1, :], U32)

    def main_unit(kv, hh, r0, n, tiles, pcs):
        c0, c1 = 128 * tiles[0], 128 * tiles[-1] + 128
        lhs = _unpack(tie_rows(l_refs[kv][hh, r0 // 2:(r0 + n) // 2, :], pcs))
        m_ = _dot_t(lhs, _unpack(r_rows(kv, hh, c0, c1)))
        if kv == 0:
            m_ = m_ * scales[0]
        nlo = min(r0 + n, DM) - r0
        for j in tiles:
            blk = m_[:, 128 * j - c0:128 * j - c0 + 128]
            if nlo > 0:
                col = (j * H + hh) * 128
                w_refs[kv][r0 // 2:(r0 + nlo) // 2, col:col + 128] = _pack(blk[:nlo])
            if r0 + n == D:
                hr_ref[kv, 32 * hh:32 * hh + 32, 128 * j:128 * j + 128] = _pack(blk[DM - r0:])

    def main_units(kv, heads, r0, n, tiles):
        return [(max(n, 64) * len(tiles) // 2,
                 functools.partial(main_unit, kv, hh, r0, n, tiles)) for hh in heads]

    def tt_unit(kv, hh, tiles, pcs):
        c0, c1 = FT[tiles[0]][0], FT[tiles[-1]][0] + FT[tiles[-1]][1]
        lhs = _unpack(tie_rows(r_rows(kv, hh, DM, D), pcs))
        m_ = _dot_t(lhs, _unpack(l_refs[kv][hh, c0 // 2:c1 // 2, :]))
        if kv == 0:
            m_ = m_ * scales[0]
        tt_ref[kv, 32 * hh:32 * hh + 32, c0:c1] = _pack(m_)

    def tt_units(kv, heads, tiles):
        return [(32 * len(tiles), functools.partial(tt_unit, kv, hh, tiles)) for hh in heads]

    def tt_piece(kv, hp, j):
        v = tt_ref[kv, 64 * hp:64 * hp + 64, 128 * j:128 * j + 128]
        if j == 3 and kv == 0:
            v = jnp.where(lo32, v[:32], _roll(v[32:], DH))
            wG_ref[DM // 2:, 128 * hp:128 * hp + 128] = v
            return _or8(v)
        v = pltpu.bitcast(_unpack(v).T, U32)
        if j < 3:
            col = (3 * H + hp) * 128
            w_refs[kv][64 * j:64 * j + 64, col:col + 128] = v
        else:
            v = v[:32]
            zero = jnp.zeros_like(v)
            hr_ref[kv, 64 * hp:64 * hp + 64, DM:DX] = jnp.concatenate(
                [jnp.where(lo32, v, zero), jnp.where(lo32, zero, v)], axis=0)
        return _or8(v)

    def tt_pieces(kv, pairs, tiles):
        return [functools.partial(tt_piece, kv, hp, j) for hp in pairs for j in tiles]

    def wg_piece(hp, j):
        v = pltpu.bitcast(_unpack(hr_ref[0, 64 * hp:64 * hp + 64, 128 * j:128 * j + 128]).T, U32)
        wG_ref[64 * j:64 * j + 64, 128 * hp:128 * hp + 128] = v
        return _or8(v)

    def mod_unit(c0, c1, pcs):
        assert not pcs
        cc = c_ref[...].astype(F32)
        sc = jnp.broadcast_to(cc * jax.nn.sigmoid(cc), (8, D)).astype(BF16)
        mod_ref[:, c0:c1] = _r(_dot(sc, wmod_ref[:, c0:c1]))

    def mod_units(c0, c1):
        return [(0, functools.partial(mod_unit, a, min(a + 256, c1))) for a in range(c0, c1, 256)]

    def col_piece(i, j):
        f0, n = FT[j]
        if i < 6:
            v = mod_ref[0:1, :][:, i * D + f0:i * D + f0 + n]
            if i in (1, 4):
                v = _r(1.0 + v)
        else:
            v = wr_ref[...].astype(F32).reshape(1, D)[:, f0:f0 + n]
        cl = jnp.broadcast_to(v, (TB, n)).T
        col_ref[i, f0:f0 + n] = cl
        return _fold8(cl)

    def col_pieces(idx):
        return [functools.partial(col_piece, i, j) for i in idx for j in range(4)]

    def stats_mean(acc):
        return jnp.sum(acc, axis=0, keepdims=True) * (1.0 / D)

    def stats_inv(acc):
        var = jnp.sum(acc, axis=0, keepdims=True) * (1.0 / D)
        return 1.0 / _r(jnp.sqrt(_r(_r(var) + EPS)))

    def ln1_pieces(b):
        t0 = b * TB if isinstance(b, int) else pl.multiple_of(b * TB, TB)
        st = {}

        def load(k):
            f0, n = FT[k]
            return xt_ref[f0:f0 + n, pl.ds(t0, TB)].astype(F32)

        def p1(k):
            s_ = _fold8(load(k))
            st['s'] = s_ if k == 0 else st['s'] + s_
            return st['s']

        def p2(k):
            if k == 0:
                st['mean'] = stats_mean(st['s'])
            xc = load(k) - st['mean']
            s_ = _fold8(xc * xc)
            st['q'] = s_ if k == 0 else st['q'] + s_
            return st['q']

        def p3(k):
            if k == 0:
                st['inv'] = stats_inv(st['q'])
                st['m'] = _r(st['mean'])
            f0, n = FT[k]
            h = (load(k) - st['m']) * st['inv'] * col_ref[1, f0:f0 + n] + col_ref[0, f0:f0 + n]
            if n < 128:
                h = jnp.concatenate([h, h], axis=0)
            ht = h.T
            h_ref[pl.ds(t0, TB), 128 * k:128 * k + 128] = ht
            return _fold8(ht)

        return [functools.partial(f, k) for f in (p1, p2, p3) for k in range(4)]

    def post_pieces(b):
        if isinstance(b, int):
            t0, r0 = b * TB, b * (TB // 2)
        else:
            t0, r0 = pl.multiple_of(b * TB, TB), pl.multiple_of(b * (TB // 2), TB // 2)
        st = {}

        def p1(k):
            f0, n = FT[k]
            a = _unpack(a_ref[pl.ds(r0, TB // 2), 128 * k:128 * k + 128]).T[:n].astype(F32)
            x = xt_ref[f0:f0 + n, pl.ds(t0, TB)].astype(F32)
            x1 = _r(x + col_ref[2, f0:f0 + n] * a)
            x1_ref[f0:f0 + n, pl.ds(t0, TB)] = x1
            s_ = _fold8(x1)
            st['s'] = s_ if k == 0 else st['s'] + s_
            return st['s']

        def p2(k):
            if k == 0:
                st['mean'] = stats_mean(st['s'])
            f0, n = FT[k]
            xc = x1_ref[f0:f0 + n, pl.ds(t0, TB)] - st['mean']
            s_ = _fold8(xc * xc)
            st['q'] = s_ if k == 0 else st['q'] + s_
            return st['q']

        def p3(k):
            if k == 0:
                st['inv'] = stats_inv(st['q'])
                st['m'] = _r(st['mean'])
            f0, n = FT[k]
            x1 = x1_ref[f0:f0 + n, pl.ds(t0, TB)]
            h2 = ((x1 - st['m']) * st['inv'] * col_ref[4, f0:f0 + n]
                  + col_ref[3, f0:f0 + n]).astype(BF16)
            h2_ref[f0 // 2:(f0 + n) // 2, pl.ds(t0, TB)] = pltpu.bitcast(h2, U32)
            h2 = h2.astype(F32)
            s_ = _fold8(h2 * col_ref[6, f0:f0 + n])
            st['r'] = s_ if k == 0 else st['r'] + s_
            ot_ref[f0:f0 + n, pl.ds(t0, TB)] = (x1 + col_ref[5, f0:f0 + n] * h2).astype(BF16)
            if k == 3:
                r_ref[pl.ds(b, 1), :] = _r(jnp.sum(st['r'], axis=0, keepdims=True))
            return st['r']

        return [functools.partial(f, k) for f in (p1, p2, p3) for k in range(4)]

    lane40 = lax.broadcasted_iota(jnp.int32, (M + SEG, 128), 1)
    tri = lax.broadcasted_iota(jnp.int32, (8, 128), 0) >= (lane8 & 7)
    bits40 = [(lane40 & (16 << b)) != 0 for b in range(3)]

    def blocksel(srcs):
        for b in range(3):
            nxt = []
            for u, v in zip(srcs[0::2], srcs[1::2]):
                nxt.append(v if u is None else u if v is None else jnp.where(bits40[b], v, u))
            srcs = nxt
        return srcs[0]

    def stack4(y, g):
        return jnp.concatenate(
            [y[8 * g:8 * g + 8, 128 * t:128 * t + 128] for t in range(4)], axis=0)

    def proj_chunk(lhs, kv, jc, dests, pcs):
        j, c = jc
        toks = [pltpu.bitcast(pc(), U32) for pc in pcs]
        tok = functools.reduce(jnp.bitwise_or, toks) if toks else None
        if kv == 2:
            y = _dot(lhs, _unpack(tie(wG_ref[:, 512 * c:512 * c + 512], tok)))
            g0 = 0
            if dests[0][0] is st_ref:
                for t in range(4):
                    hp = 4 * c + t
                    g_ref[16 * hp:16 * hp + 16, :] = _pack(y[:32, 128 * t:128 * t + 128])
                g0 = 4
            for g in range(g0, len(dests)):
                gn_ref[dests[g][1], 16 * c:16 * c + 16, :] = _pack(stack4(y, g))
            return
        c0 = (j * H + 4 * c) * 128
        y = _dot(lhs[:, :DM], _unpack(tie(w_refs[kv][:, c0:c0 + 512], tok)))
        for g, (ref, gi) in enumerate(dests):
            if j < 3:
                ref[kv, gi, 16 * c:16 * c + 16, 128 * j:128 * j + 128] = _pack(stack4(y, g))
            else:
                parts = []
                for t in range(4):
                    v = y[8 * g:8 * g + 8, 128 * t:128 * t + 128]
                    parts += [jnp.where(lo_half, v, 0.0), jnp.where(lo_half, 0.0, v)]
                ref[kv, gi, 32 * c:32 * c + 32, DM:DX] = _pack(jnp.concatenate(parts, axis=0))

    chunks = [(3, 0), (3, 1)] + [(j, c) for j in range(3) for c in range(4)]
    gchunks = [(0, 0), (0, 1)]
    own = [(st_ref, g) for g in range(4)]
    xdst = [(xn_ref, k) for k in range(4)]

    def x_lhs(b):
        t0 = b * TB if isinstance(b, int) else pl.multiple_of(b * TB, TB)
        rows = [h_ref[pl.ds(t0 + SEG * k + POS[4], 8), :] for k in range(4)]
        return jnp.concatenate(rows, axis=0).astype(BF16)[:, :D]

    def sq(j):
        return swap_pieces(rq_ref, tq_ref, *FT[j])

    def sk(j):
        return swap_pieces(rk_ref, tk_ref, *FT[j])

    def mix(a, b):
        out = []
        for i, u in enumerate(a):
            out.append(u)
            out += b[(i * len(b)) // len(a):((i + 1) * len(b)) // len(a)]
        return out

    allh = range(H)
    lo3, all4 = [0, 1, 2], [0, 1, 2, 3]

    def vfull(heads):
        return mix(main_units(1, heads, 0, D, lo3), tt_units(1, heads, all4))

    with _scope('V0'):
        v_cp[0].wait()
        swap(rv_ref, tv_ref, 0, 64)
        o_cp[0].wait()
        for i in range(6):
            v_cp[i + 1].wait()
            region(main_units(1, range(8), 64 * i, 64, lo3),
                   swap_pieces(rv_ref, tv_ref, 64 * (i + 1), 64), skip=96)
        region(main_units(1, range(8), DM, 64, lo3) + tt_units(1, range(8), all4))
    with _scope('V1'):
        o_cp[1].wait()
        region(vfull(range(8, 12)), tt_pieces(1, range(4), all4))
    with _scope('V2'):
        o_cp[2].wait()
        q_cp[0].wait()
        region(vfull(range(12, 14)), sq(0))
    with _scope('V3'):
        k_cp[0].wait()
        region(vfull(range(14, 16)), sk(0))
    with _scope('K0'):
        k_cp[1].wait()
        region(main_units(0, allh, 0, 128, [0]), sk(1), skip=64)
    with _scope('K1'):
        q_cp[1].wait()
        region(main_units(0, allh, 128, 128, [0]), sq(1), skip=64)
    with _scope('K2'):
        q_cp[3].wait()
        region(main_units(0, allh, 0, 256, [1]), mix(sq(3), tt_pieces(1, range(4, 8), all4)))
    with _scope('K3'):
        k_cp[2].wait()
        region(tt_units(0, allh, [0, 1]), sk(2), skip=64)
    with _scope('K4'):
        q_cp[2].wait()
        region(mix(main_units(0, allh, 256, 128, [0, 1]), tt_units(0, allh, [2])),
               mix(sq(2), tt_pieces(0, range(8), [0, 1])))
    with _scope('K5'):
        k_cp[3].wait()
        x_cp[0].wait()
        mod_cp[0].wait()
        u = main_units(0, allh, 0, DM, [2])
        l0 = ln1_pieces(0)
        region(mix(u[:4], mod_units(0, MODA)) + u[4:],
               mix(sk(3), l0[:8]) + tt_pieces(0, range(8), [2]) + col_pieces([0, 1]))
    with _scope('K6'):
        region(mix(main_units(0, allh, DM, 64, lo3), tt_units(0, allh, [3])),
               l0[8:] + ln1_pieces(1))
    with _scope('x0'):
        mod_cp[1].wait()
        xl0 = x_lhs(0)
        jobs = ([(1, jc) for jc in chunks] + [(0, jc) for jc in chunks[2:] + chunks[:2]]
                + [(2, jc) for jc in gchunks])
        units = [(96, functools.partial(proj_chunk, xl0, kv, jc, xdst)) for kv, jc in jobs]
        wgp = ([functools.partial(wg_piece, hp, j) for hp in range(8) for j in range(3)]
               + tt_pieces(0, range(8), [3]))
        region(mix(units[:7], mod_units(MODA, 6 * D)) + units[7:26],
               wgp[:12] + mix(wgp[12:], col_pieces([2, 3, 4, 5, 6])), skip=96)
        region(units[26:])
        x_cp[1].wait()
        for cp in mlp_cp:
            cp.start()

    def segment(k, hf, r0, sched, xl, ride, fill):
        final = not isinstance(k, int)
        ks = 0 if final else k
        xs_ref, gs_ref = (xn_ref, gn_ref) if final else (xc_ref, gc_ref)
        hq = jnp.concatenate([hf, jnp.zeros((8, DX), F32)], axis=0).astype(BF16)
        lhs = hq[:32, :D]
        lhs_x = None if xl is None else jnp.concatenate([lhs, xl], axis=0)

        def nextp():
            pc = sched.pop(0) if sched else None
            return [] if pc is None else [pc]

        def chunk(kv, jc):
            if xl is not None and (kv, jc) in ride:
                proj_chunk(lhs_x, kv, jc, own + xdst, nextp())
            else:
                proj_chunk(lhs, kv, jc, own, nextp())

        def filler(n):
            for _ in range(n):
                if xl is not None and fill:
                    kv, jc = fill.pop(0)
                    proj_chunk(xl, kv, jc, xdst, nextp())

        parts = []
        for g in range(5):
            v = hf[8 * g:8 * g + 8, DM:]
            parts += [jnp.where(lo_half, v, 0.0), jnp.where(lo_half, 0.0, v)]
        b0 = jnp.concatenate(parts + [jnp.zeros((48, 128), F32)], axis=0).astype(BF16)

        for jc in gchunks:
            chunk(2, jc)
        for n_, jc in enumerate(chunks):
            chunk(0, jc)
            if n_ == 2:
                lg = _unpack(jnp.concatenate([g_ref[...], gs_ref[k]], axis=0))
                tt = jnp.concatenate(
                    [_dot_t(lg[80 * i:80 * i + 80], b0) for i in range(4)], axis=0)
                rr = [_roll(jnp.concatenate([tt[32 * hp:32 * hp + 32],
                                             tt[256 + 8 * hp:264 + 8 * hp]], axis=0), 16 * hp)
                      for hp in range(8)]
                s2 = [_roll(blocksel([rr[(b - g) % 8] for b in range(8)]), -16 * g)
                      for g in range(5)]
        lead = chunks[3 * ks:3 * ks + 3]
        vorder = lead + [jc for jc in chunks if jc not in lead]
        sc = {}
        chunk(1, vorder[0])
        for n_, g in enumerate((4, 0, 1, 2, 3)):
            kst = _unpack(xs_ref[0, k] if g == 4 else st_ref[0, g])
            sg = _dot_t(hq[:16 * QROWS[g]], kst)
            for q in range(5):
                if (q, g) not in VIS:
                    continue
                v = _r(sg[8 * q:8 * q + 8] + s2[g][8 * q:8 * q + 8])
                if q == g and g > 0:
                    v = jnp.where(tri, v, -1e9)
                sc[q, g] = v
            if n_ in (1, 3):
                chunk(1, vorder[(n_ + 1) // 2])
        per_q = [[g for g in range(5) if (q, g) in VIS] for q in range(5)]
        mx = jnp.concatenate([functools.reduce(jnp.maximum, [sc[q, g] for g in per_q[q]])
                              for q in range(5)], axis=0)
        mx = _group8_reduce(mx, jnp.maximum, lane40)
        ex = {qg: jnp.exp(v - mx[8 * qg[0]:8 * qg[0] + 8]) for qg, v in sc.items()}
        den = jnp.concatenate([functools.reduce(jnp.add, [ex[q, g] for g in per_q[q]])
                               for q in range(5)], axis=0)
        inv = 1.0 / _group8_reduce(den, jnp.add, lane40)
        zero8 = jnp.zeros((8, 128), F32)
        pg = [jnp.concatenate([ex[q, g] * inv[8 * q:8 * q + 8] if (q, g) in VIS else zero8
                               for q in range(5)], axis=0) for g in range(5)]
        pb = [jnp.concatenate([v, zero8], axis=0).astype(BF16) for v in pg]
        for jc in vorder[3:]:
            chunk(1, jc)
        filler(NFILL[0])
        outs = {}

        def out_main(j):
            cols = slice(128 * j, 128 * j + 128)
            v04 = jnp.concatenate([st_ref[1, 0, :, cols], xs_ref[1, k, :, cols]], axis=0)
            o3 = _dot(jnp.concatenate([pb[0], pb[4]], axis=1), _unpack(v04))
            v23 = jnp.concatenate([st_ref[1, 2, :, cols], st_ref[1, 3, :, cols]], axis=0)
            o2 = _dot(jnp.concatenate([pb[2][:32], pb[3][:32]], axis=1), _unpack(v23))
            o1 = _dot(pb[1][:16], _unpack(st_ref[1, 1, :, cols]))
            outs[j] = jnp.concatenate(
                [o3[:16] + o2[:16] + o1, o3[16:32] + o2[16:32], o3[32:40]], axis=0)

        for j in (3, 0, 1):
            out_main(j)
        filler(NFILL[1])
        pr = [_roll(pg[g], 16 * g) for g in range(5)]
        lz = jnp.concatenate(
            [_roll(blocksel([pr[(b - hp) % 8] if (b - hp) % 8 < 5 else None for b in range(8)]),
                   -16 * hp) for hp in range(8)], axis=0).astype(BF16)
        zt = [_dot(lz[80 * i:80 * i + 80], b0) for i in range(4)]
        zq = jnp.concatenate([zt[hp // 2][40 * (hp % 2):40 * (hp % 2) + 40]
                              for hp in range(8)], axis=1)
        if final:
            zq = jnp.concatenate([zq, jnp.zeros((8, 64 * H), F32)], axis=0).astype(BF16)
            nr = M + SEG
        else:
            zd_ref[k] = zq[32:]
            zq = zq[:32].astype(BF16)
            nr = 32
        out_main(2)
        filler(NFILL[2])
        for j in (3, 0, 1, 2):
            o2 = outs[j][:nr] + _dot(zq, _unpack(hr_ref[1, :, 128 * j:128 * j + 128]))[:nr]
            if not final:
                od_ref[k, 0:8, 128 * j:128 * j + 128] = outs[j][32:]
            outs[j] = o2
        filler(NFILL[3] if ks < 3 else NFILL[4])
        hi = outs[3] + _roll(outs[3], DH)
        o = jnp.concatenate([outs[0], outs[1], outs[2], hi], axis=1)
        if final:
            a_ref[pl.ds(r0, 16), :] = _pack(jnp.concatenate([o[32:], o[16:32], o[8:16]], axis=0))
        else:
            od_ref[k, 8:16, :] = o[16:24]
            a_ref[pl.ds(r0 + 8, 8), :] = _pack(jnp.concatenate([o[24:32], o[8:16]], axis=0))
        return _r(o[:M])

    def deferred(b):
        zq = zd_ref[...].reshape(32, 64 * H).astype(BF16)
        o2 = [_dot(zq, _unpack(hr_ref[1, :, 128 * j:128 * j + 128])) for j in range(4)]
        for k in range(4):
            t = [o2[j][8 * k:8 * k + 8] + od_ref[k, 0:8, 128 * j:128 * j + 128] for j in range(4)]
            t[3] = t[3] + _roll(t[3], DH)
            rows = jnp.concatenate([jnp.concatenate(t, axis=1), od_ref[k, 8:16, :]], axis=0)
            ra = b * (TB // 2) + k * (SEG // 2)
            if not isinstance(b, int):
                ra = pl.multiple_of(ra, SEG // 2)
            a_ref[pl.ds(ra, 8), :] = _pack(rows)

    def seg_rows(mem, r0):
        return jnp.concatenate([mem, h_ref[pl.ds(r0 + 24, 8), :], h_ref[pl.ds(r0 + 8, 16), :],
                                h_ref[pl.ds(r0, 8), :]], axis=0)

    def block(i, mem):
        prev = jnp.maximum(i - 1, 0)
        sched = []
        for u, v in zip(post_pieces(prev), ln1_pieces(jnp.minimum(i + 2, NB - 1))):
            sched += [None, None, None, v, None, None, None, u]
        xl = x_lhs(i + 1)
        deferred(prev)
        xc_ref[...] = xn_ref[...]
        gc_ref[...] = gn_ref[...]
        nfill = 4 * sum(NFILL[:3]) + 3 * NFILL[3] + NFILL[4]
        alljobs = ([(0, jc) for jc in chunks] + [(1, jc) for jc in chunks[12:]]
                   + [(2, jc) for jc in gchunks])
        fill, rest = alljobs[:nfill], alljobs[nfill:]
        for k in range(4):
            ride = [(1, jc) for jc in chunks[3 * k:3 * k + 3]] + rest[k::4]
            r0 = pl.multiple_of(i * TB + k * SEG, SEG)
            ra = pl.multiple_of(i * (TB // 2) + k * (SEG // 2), SEG // 2)
            mem = segment(k, seg_rows(mem, r0), ra, sched, xl, ride, fill)
        assert not any(sched) and not fill
        return mem

    def last_segment(k, mem):
        r0 = pl.multiple_of((NB - 1) * TB + k * SEG, SEG)
        ra = pl.multiple_of((NB - 1) * (TB // 2) + k * (SEG // 2), SEG // 2)
        return segment(k, seg_rows(mem, r0), ra, [], None, (), [])

    m0 = mem0_ref[0].astype(F32)
    m0 = jnp.concatenate([m0, m0[:, DM:]], axis=1)
    with _scope('main'):
        mem = lax.fori_loop(0, NB - 1, block, m0)
    nfull = (NB - 2) * TB
    out_a = copy(ot_ref.at[:, pl.ds(0, nfull)], o_hbm.at[0, :, pl.ds(0, nfull)])
    out_a.start()
    deferred(NB - 2)
    with _scope('last'):
        lax.fori_loop(0, 4, last_segment, mem)

    for cp in mlp_cp:
        cp.wait()
    out_a.wait()
    for pa, pb in zip(post_pieces(NB - 2), post_pieces(NB - 1)):
        pa()
        pb()
    out_b = copy(ot_ref.at[:, pl.ds(nfull, 2 * TB)], o_hbm.at[0, :, pl.ds(nfull, 2 * TB)])
    out_b.start()

    bits = pltpu.bitcast(r_ref[...] + 0.0, jnp.int32)
    bits = jnp.where(bits < 0, bits ^ jnp.int32(0x7FFF0000), bits)
    tok = (lax.broadcasted_iota(jnp.int32, (NB, TB), 0) * TB
           + lax.broadcasted_iota(jnp.int32, (NB, TB), 1))
    idx = (S - 1) - (jnp.max(bits | ((S - 1) - tok)) & (S - 1))
    blk = idx // TB
    ln = idx - blk * TB
    t0 = pl.multiple_of(blk * TB, TB)
    h2 = _unpack(h2_ref[:, pl.ds(t0, TB)])
    onehot = (lax.broadcasted_iota(jnp.int32, (8, TB), 1) == ln)
    hsel = _dot_t(onehot.astype(BF16), h2).astype(BF16)
    gt = _r(_dot(hsel, wg_ref[...]))
    gt = _r(gt * jax.nn.sigmoid(gt))
    up = _r(_dot(hsel, wu_ref[...]))
    y = _r(_dot_t(_r(gt * up).astype(BF16), wdt_ref[...]))
    yt = jnp.broadcast_to(y[0:1], (TB, D)).T
    yt = _r(yt * _r(jax.nn.sigmoid(r_ref[pl.ds(blk, 1), :])))
    h2 = h2.astype(F32)
    sel = lax.broadcasted_iota(jnp.int32, (D, TB), 1) == ln
    hb2 = jnp.where(sel, _r(h2 + yt), h2)
    fix = (x1_ref[:, pl.ds(t0, TB)] + col_ref[5] * hb2).astype(BF16)
    out_b.wait()
    ot_ref[:, pl.ds(t0, TB)] = fix
    out_c = copy(ot_ref.at[:, pl.ds(t0, TB)], o_hbm.at[0, :, pl.ds(t0, TB)])
    out_c.start()
    out_c.wait()


@jax.jit
def pallas_adaLN_cond__memory_aug_recurrent_mem_tr__moe_arch_mod__prompt_kernel(A_x, A_mem0, A_Wq, A_Wk, A_Wv, A_Wo, A_seg_len, B_x, B_w_r, B_w_gate, B_w_up,
              B_w_down, c, w_mod):
    any_spec = pl.BlockSpec(memory_space=pl.ANY)
    vmem_spec = pl.BlockSpec(memory_space=pltpu.VMEM)
    out_t = pl.pallas_call(
        _kernel,
        out_shape=jax.ShapeDtypeStruct((1, D, S), BF16),
        in_specs=[any_spec, vmem_spec, any_spec, any_spec, any_spec, any_spec, vmem_spec,
                  any_spec, any_spec, any_spec, vmem_spec, any_spec],
        out_specs=any_spec,
        scratch_shapes=[
            pltpu.VMEM((D, S), BF16),
            pltpu.VMEM((D, H, E), BF16),
            pltpu.VMEM((D, H, E), BF16),
            pltpu.VMEM((D, H, E), BF16),
            pltpu.VMEM((H, D, E), BF16),
            pltpu.VMEM((D, FF), BF16),
            pltpu.VMEM((D, FF), BF16),
            pltpu.VMEM((D, FF), BF16),
            pltpu.VMEM((D, 6 * D), BF16),
            pltpu.VMEM((D, S), BF16),
            pltpu.VMEM((S, DX), F32),
            pltpu.VMEM((S // 2, DX), U32),
            pltpu.VMEM((H, D // 2, E), U32),
            pltpu.VMEM((H, D // 2, E), U32),
            pltpu.VMEM((H, D // 2, E), U32),
            pltpu.VMEM((DM // 2, NT * 128), U32),
            pltpu.VMEM((DM // 2, NT * 128), U32),
            pltpu.VMEM((2, 4, 64, DX), U32),
            pltpu.VMEM((2, 4, 64, DX), U32),
            pltpu.VMEM((2, 4, 64, DX), U32),
            pltpu.VMEM((2, 32 * H, DX), U32),
            pltpu.VMEM((2, 32 * H, DX), U32),
            pltpu.VMEM((D // 2, 64 * H), U32),
            pltpu.VMEM((128, 128), U32),
            pltpu.VMEM((4, 32, 128), U32),
            pltpu.VMEM((4, 32, 128), U32),
            pltpu.VMEM((4, 8, 64 * H), F32),
            pltpu.VMEM((4, 16, DX), F32),
            pltpu.VMEM((8, 6 * D), F32),
            pltpu.VMEM((7, D, TB), F32),
            pltpu.VMEM((NB, TB), F32),
            pltpu.VMEM((D, S), F32),
            pltpu.VMEM((D // 2, S), U32),
            pltpu.VMEM((8, 128), U32),
            pltpu.SemaphoreType.DMA((32,)),
        ],
        compiler_params=pltpu.CompilerParams(vmem_limit_bytes=120 * 1024 * 1024),
    )(jnp.swapaxes(A_x, 1, 2), A_mem0, A_Wq, A_Wk, A_Wv, jnp.swapaxes(A_Wo, 1, 2),
      B_w_r, B_w_gate, B_w_up, B_w_down.T, c, w_mod)
    return jnp.swapaxes(out_t, 1, 2)
```

```python
import functools

import jax
import jax.numpy as jnp
from jax import lax
import jax.experimental.pallas as pl
import jax.experimental.pallas.tpu as pltpu

F32 = jnp.float32
BF16 = jnp.bfloat16
U32 = jnp.uint32

S, D, H, E, M, SEG, FF = 2048, 448, 16, 256, 8, 32, 1792
DM = 384
DH = D - DM
DX = 512
NT = 56
EPS = 1e-5
TB = 128
NB = S // TB
NFILL = (0, 1, 1, 1, 1)

POS = (None, 24, 8, 16, 0)
VIS = frozenset((q, g) for q in range(5) for g in range(5)
                if q == 0 or g == 0 or POS[q] >= POS[g])
QROWS = [1 + max(q // 2 for q in range(5) if (q, g) in VIS) for g in range(5)]
FT = [(0, 128), (128, 128), (256, 128), (384, 64)]
MODA = 2 * D


def _r(x):
    return x.astype(BF16).astype(F32)


def _dot(a, b):
    return jnp.dot(a, b, preferred_element_type=F32)


def _dot_t(a, b):
    return lax.dot_general(a, b, (((1,), (1,)), ((), ())), preferred_element_type=F32)


def _pack(x):
    return pltpu.bitcast(x.astype(BF16), U32)


def _unpack(x):
    return pltpu.bitcast(x, BF16)


def _fold8(v):
    return jnp.sum(v.reshape(v.shape[0] // 8, 8, v.shape[1]), axis=0)


def _or8(v):
    return functools.reduce(jnp.bitwise_or, [v[8 * i:8 * i + 8] for i in range(v.shape[0] // 8)])


def _roll(v, s):
    s = s % 128
    return pltpu.roll(v, s, 1) if s else v


def _group8_reduce(v, op, lane):
    for d in (1, 2, 4):
        v = op(v, jnp.where((lane & d) != 0, _roll(v, d), _roll(v, -d)))
    return v


def _kernel(xt_hbm, mem0_hbm, wq_hbm, wk_hbm, wv_hbm, wot_hbm, wr_hbm, wg_hbm, wu_hbm, wdt_hbm,
            c_hbm, wmod_hbm, o_hbm,
            mem0_ref, wr_ref, c_ref, xt_ref, rq_ref, rk_ref, rv_ref, wot_ref,
            wg_ref, wu_ref, wdt_ref, wmod_ref, ot_ref,
            h_ref, a_ref, tq_ref, tk_ref, tv_ref, wK_ref, wV_ref, st_ref, xc_ref, xn_ref,
            hr_ref, tt_ref, wG_ref, g_ref, gc_ref, gn_ref, zd_ref, od_ref, mod_ref, col_ref,
            r_ref, x1_ref, h2_ref, z_ref, sems):
    nsem = [0]

    def copy(src, dst):
        nsem[0] += 1
        return pltpu.make_async_copy(src, dst, sems.at[nsem[0] - 1])

    def rows_copy(src, dst, r0, n):
        return copy(src.at[pl.ds(r0, n)], dst.at[pl.ds(r0, n)])

    def cols_copy(src, dst, c0, n):
        return copy(src.at[:, pl.ds(c0, n)], dst.at[:, pl.ds(c0, n)])

    o_cp = [rows_copy(wot_hbm, wot_ref, a, b - a) for a, b in ((0, 8), (8, 12), (12, 16))]
    v_cp = [rows_copy(wv_hbm, rv_ref, 64 * i, 64) for i in range(7)]
    q_cp = [rows_copy(wq_hbm, rq_ref, f0, n) for f0, n in FT]
    k_cp = [rows_copy(wk_hbm, rk_ref, f0, n) for f0, n in FT]
    mod_cp = [cols_copy(wmod_hbm, wmod_ref, 0, MODA),
              cols_copy(wmod_hbm, wmod_ref, MODA, 6 * D - MODA)]
    x_cp = [cols_copy(xt_hbm.at[0], xt_ref, 0, 2 * TB),
            cols_copy(xt_hbm.at[0], xt_ref, 2 * TB, S - 2 * TB)]
    mlp_cp = [copy(wg_hbm, wg_ref), copy(wu_hbm, wu_ref), copy(wdt_hbm, wdt_ref)]
    small_cp = [copy(mem0_hbm, mem0_ref), copy(wr_hbm, wr_ref), copy(c_hbm, c_ref)]
    for cp in ([o_cp[0]] + v_cp + small_cp + o_cp[1:]
               + [q_cp[0], k_cp[0], k_cp[1], q_cp[1], q_cp[3], k_cp[2], q_cp[2], k_cp[3]]
               + [x_cp[0], mod_cp[0], mod_cp[1], x_cp[1]]):
        cp.start()

    z_ref[...] = jnp.zeros((8, 128), U32)
    a_ref[0:TB // 2, :] = jnp.zeros((TB // 2, DX), U32)
    tt_ref[:, :, DM:DX] = jnp.zeros((2, 32 * H, 128), U32)

    lane8 = lax.broadcasted_iota(jnp.int32, (8, 128), 1)
    lo_half = lane8 < DH
    lo32 = lax.broadcasted_iota(jnp.int32, (32, 128), 1) < DH
    w_refs = (wK_ref, wV_ref)
    l_refs = (tk_ref, tv_ref)
    scales = (E ** -0.5, 1.0)

    def tie(w, tok):
        if tok is None:
            return w
        w00 = w[0:8, 0:128] | (pltpu.bitcast(tok, U32) & z_ref[...])
        top = jnp.concatenate([w00, w[0:8, 128:]], axis=1)
        return jnp.concatenate([top, w[8:]], axis=0) if w.shape[0] > 8 else top

    def tie_rows(w, pcs):
        if not pcs:
            return w
        ng = w.shape[0] // 8
        slots = {}
        for k, pc in enumerate(pcs):
            slots.setdefault((k * ng) // len(pcs) * 8, []).append(pc)
        cuts = sorted(slots) + [ng * 8]
        out = []
        for a, b in zip(cuts[:-1], cuts[1:]):
            tok = functools.reduce(jnp.bitwise_or, [pltpu.bitcast(pc(), U32) for pc in slots[a]])
            out.append(tie(w[a:b], tok))
        return jnp.concatenate(out, axis=0)

    def region(units, pieces=(), skip=200):
        total = sum(c for c, _ in units)
        pieces = list(pieces)
        n, t, done = len(pieces), 0, 0
        for cost, fn in units:
            t += cost
            upto = n if t == total else max(0, (n * (t - skip)) // (total - skip))
            fn(pieces[done:upto])
            done = max(done, upto)

    def swap(raw_ref, t_ref, r0, n):
        v = pltpu.bitcast(jnp.swapaxes(raw_ref[r0:r0 + n], 0, 1), U32)
        t_ref[:, r0 // 2:(r0 + n) // 2, :] = v

    def swap_small(raw_ref, t_ref, r0, h0, c0):
        v = pltpu.bitcast(jnp.swapaxes(raw_ref[r0:r0 + 16, h0:h0 + 8, c0:c0 + 128], 0, 1), U32)
        t_ref[h0:h0 + 8, r0 // 2:r0 // 2 + 8, c0:c0 + 128] = v
        return functools.reduce(jnp.bitwise_or, [v[i] for i in range(8)])

    def swap_pieces(raw_ref, t_ref, r0, n):
        return [functools.partial(swap_small, raw_ref, t_ref, r, h0, c0)
                for r in range(r0, r0 + n, 16) for h0 in (0, 8) for c0 in (0, 128)]

    def r_rows(kv, hh, c0, c1):
        if kv == 0:
            return tq_ref[hh, c0 // 2:c1 // 2, :]
        return pltpu.bitcast(wot_ref[hh, c0:c1, :], U32)

    def main_unit(kv, hh, r0, n, tiles, pcs):
        c0, c1 = 128 * tiles[0], 128 * tiles[-1] + 128
        lhs = _unpack(tie_rows(l_refs[kv][hh, r0 // 2:(r0 + n) // 2, :], pcs))
        m_ = _dot_t(lhs, _unpack(r_rows(kv, hh, c0, c1)))
        if kv == 0:
            m_ = m_ * scales[0]
        nlo = min(r0 + n, DM) - r0
        for j in tiles:
            blk = m_[:, 128 * j - c0:128 * j - c0 + 128]
            if nlo > 0:
                col = (j * H + hh) * 128
                w_refs[kv][r0 // 2:(r0 + nlo) // 2, col:col + 128] = _pack(blk[:nlo])
            if r0 + n == D:
                hr_ref[kv, 32 * hh:32 * hh + 32, 128 * j:128 * j + 128] = _pack(blk[DM - r0:])

    def main_units(kv, heads, r0, n, tiles):
        return [(max(n, 64) * len(tiles) // 2,
                 functools.partial(main_unit, kv, hh, r0, n, tiles)) for hh in heads]

    def tt_unit(kv, hh, tiles, pcs):
        c0, c1 = FT[tiles[0]][0], FT[tiles[-1]][0] + FT[tiles[-1]][1]
        lhs = _unpack(tie_rows(r_rows(kv, hh, DM, D), pcs))
        m_ = _dot_t(lhs, _unpack(l_refs[kv][hh, c0 // 2:c1 // 2, :]))
        if kv == 0:
            m_ = m_ * scales[0]
        tt_ref[kv, 32 * hh:32 * hh + 32, c0:c1] = _pack(m_)

    def tt_units(kv, heads, tiles):
        return [(32 * len(tiles), functools.partial(tt_unit, kv, hh, tiles)) for hh in heads]

    def tt_piece(kv, hp, j):
        v = tt_ref[kv, 64 * hp:64 * hp + 64, 128 * j:128 * j + 128]
        if j == 3 and kv == 0:
            v = jnp.where(lo32, v[:32], _roll(v[32:], DH))
            wG_ref[DM // 2:, 128 * hp:128 * hp + 128] = v
            return _or8(v)
        v = pltpu.bitcast(_unpack(v).T, U32)
        if j < 3:
            col = (3 * H + hp) * 128
            w_refs[kv][64 * j:64 * j + 64, col:col + 128] = v
        else:
            v = v[:32]
            zero = jnp.zeros_like(v)
            hr_ref[kv, 64 * hp:64 * hp + 64, DM:DX] = jnp.concatenate(
                [jnp.where(lo32, v, zero), jnp.where(lo32, zero, v)], axis=0)
        return _or8(v)

    def tt_pieces(kv, pairs, tiles):
        return [functools.partial(tt_piece, kv, hp, j) for hp in pairs for j in tiles]

    def wg_piece(hp, j):
        v = pltpu.bitcast(_unpack(hr_ref[0, 64 * hp:64 * hp + 64, 128 * j:128 * j + 128]).T, U32)
        wG_ref[64 * j:64 * j + 64, 128 * hp:128 * hp + 128] = v
        return _or8(v)

    def mod_unit(c0, c1, pcs):
        assert not pcs
        cc = c_ref[...].astype(F32)
        sc = jnp.broadcast_to(cc * jax.nn.sigmoid(cc), (8, D)).astype(BF16)
        mod_ref[:, c0:c1] = _r(_dot(sc, wmod_ref[:, c0:c1]))

    def mod_units(c0, c1):
        return [(0, functools.partial(mod_unit, a, min(a + 256, c1))) for a in range(c0, c1, 256)]

    def col_piece(i, j):
        f0, n = FT[j]
        if i < 6:
            v = mod_ref[0:1, i * D + f0:i * D + f0 + n]
            if i in (1, 4):
                v = _r(1.0 + v)
        else:
            v = wr_ref[...].astype(F32).reshape(1, D)[:, f0:f0 + n]
        cl = jnp.broadcast_to(v, (TB, n)).astype(BF16).T.astype(F32)
        col_ref[i, f0:f0 + n] = cl
        return _fold8(cl)

    def col_pieces(idx):
        return [functools.partial(col_piece, i, j) for i in idx for j in range(4)]

    def stats_mean(acc):
        return jnp.sum(acc, axis=0, keepdims=True) * (1.0 / D)

    def stats_inv(acc):
        var = jnp.sum(acc, axis=0, keepdims=True) * (1.0 / D)
        return 1.0 / _r(jnp.sqrt(_r(_r(var) + EPS)))

    def ln1_pieces(b):
        t0 = b * TB if isinstance(b, int) else pl.multiple_of(b * TB, TB)
        st = {}

        def load(k):
            f0, n = FT[k]
            return xt_ref[f0:f0 + n, pl.ds(t0, TB)].astype(F32)

        def p1(k):
            s_ = _fold8(load(k))
            st['s'] = s_ if k == 0 else st['s'] + s_
            return st['s']

        def p2(k):
            if k == 0:
                st['mean'] = stats_mean(st['s'])
            xc = load(k) - st['mean']
            s_ = _fold8(xc * xc)
            st['q'] = s_ if k == 0 else st['q'] + s_
            return st['q']

        def p3(k):
            if k == 0:
                st['inv'] = stats_inv(st['q'])
                st['m'] = _r(st['mean'])
            f0, n = FT[k]
            h = (load(k) - st['m']) * st['inv'] * col_ref[1, f0:f0 + n] + col_ref[0, f0:f0 + n]
            if n < 128:
                h = jnp.concatenate([h, h], axis=0)
            ht = h.astype(BF16).T.astype(F32)
            h_ref[pl.ds(t0, TB), 128 * k:128 * k + 128] = ht
            return _fold8(ht)

        return [functools.partial(f, k) for f in (p1, p2, p3) for k in range(4)]

    def post_pieces(b):
        if isinstance(b, int):
            t0, r0 = b * TB, b * (TB // 2)
        else:
            t0, r0 = pl.multiple_of(b * TB, TB), pl.multiple_of(b * (TB // 2), TB // 2)
        st = {}

        def p1(k):
            f0, n = FT[k]
            a = _unpack(a_ref[pl.ds(r0, TB // 2), 128 * k:128 * k + 128]).T[:n].astype(F32)
            x = xt_ref[f0:f0 + n, pl.ds(t0, TB)].astype(F32)
            x1 = _r(x + col_ref[2, f0:f0 + n] * a)
            x1_ref[f0:f0 + n, pl.ds(t0, TB)] = x1
            s_ = _fold8(x1)
            st['s'] = s_ if k == 0 else st['s'] + s_
            return st['s']

        def p2(k):
            if k == 0:
                st['mean'] = stats_mean(st['s'])
            f0, n = FT[k]
            xc = x1_ref[f0:f0 + n, pl.ds(t0, TB)] - st['mean']
            s_ = _fold8(xc * xc)
            st['q'] = s_ if k == 0 else st['q'] + s_
            return st['q']

        def p3(k):
            if k == 0:
                st['inv'] = stats_inv(st['q'])
                st['m'] = _r(st['mean'])
            f0, n = FT[k]
            x1 = x1_ref[f0:f0 + n, pl.ds(t0, TB)]
            h2 = ((x1 - st['m']) * st['inv'] * col_ref[4, f0:f0 + n]
                  + col_ref[3, f0:f0 + n]).astype(BF16)
            h2_ref[f0 // 2:(f0 + n) // 2, pl.ds(t0, TB)] = pltpu.bitcast(h2, U32)
            h2 = h2.astype(F32)
            s_ = _fold8(h2 * col_ref[6, f0:f0 + n])
            st['r'] = s_ if k == 0 else st['r'] + s_
            ot_ref[f0:f0 + n, pl.ds(t0, TB)] = (x1 + col_ref[5, f0:f0 + n] * h2).astype(BF16)
            if k == 3:
                r_ref[pl.ds(b, 1), :] = _r(jnp.sum(st['r'], axis=0, keepdims=True))
            return st['r']

        return [functools.partial(f, k) for f in (p1, p2, p3) for k in range(4)]

    lane40 = lax.broadcasted_iota(jnp.int32, (M + SEG, 128), 1)
    tri = lax.broadcasted_iota(jnp.int32, (8, 128), 0) >= (lane8 & 7)
    bits40 = [(lane40 & (16 << b)) != 0 for b in range(3)]

    def blocksel(srcs):
        for b in range(3):
            nxt = []
            for u, v in zip(srcs[0::2], srcs[1::2]):
                nxt.append(v if u is None else u if v is None else jnp.where(bits40[b], v, u))
            srcs = nxt
        return srcs[0]

    def stack4(y, g):
        return jnp.concatenate(
            [y[8 * g:8 * g + 8, 128 * t:128 * t + 128] for t in range(4)], axis=0)

    def proj_chunk(lhs, kv, jc, dests, pcs):
        j, c = jc
        toks = [pltpu.bitcast(pc(), U32) for pc in pcs]
        tok = functools.reduce(jnp.bitwise_or, toks) if toks else None
        if kv == 2:
            y = _dot(lhs, _unpack(tie(wG_ref[:, 512 * c:512 * c + 512], tok)))
            g0 = 0
            if dests[0][0] is st_ref:
                for t in range(4):
                    hp = 4 * c + t
                    g_ref[16 * hp:16 * hp + 16, :] = _pack(y[:32, 128 * t:128 * t + 128])
                g0 = 4
            for g in range(g0, len(dests)):
                gn_ref[dests[g][1], 16 * c:16 * c + 16, :] = _pack(stack4(y, g))
            return
        c0 = (j * H + 4 * c) * 128
        y = _dot(lhs[:, :DM], _unpack(tie(w_refs[kv][:, c0:c0 + 512], tok)))
        for g, (ref, gi) in enumerate(dests):
            if j < 3:
                ref[kv, gi, 16 * c:16 * c + 16, 128 * j:128 * j + 128] = _pack(stack4(y, g))
            else:
                parts = []
                for t in range(4):
                    v = y[8 * g:8 * g + 8, 128 * t:128 * t + 128]
                    parts += [jnp.where(lo_half, v, 0.0), jnp.where(lo_half, 0.0, v)]
                ref[kv, gi, 32 * c:32 * c + 32, DM:DX] = _pack(jnp.concatenate(parts, axis=0))

    chunks = [(3, 0), (3, 1)] + [(j, c) for j in range(3) for c in range(4)]
    gchunks = [(0, 0), (0, 1)]
    own = [(st_ref, g) for g in range(4)]
    xdst = [(xn_ref, k) for k in range(4)]

    def x_lhs(b):
        t0 = b * TB if isinstance(b, int) else pl.multiple_of(b * TB, TB)
        rows = [h_ref[pl.ds(t0 + SEG * k + POS[4], 8), :] for k in range(4)]
        return jnp.concatenate(rows, axis=0).astype(BF16)[:, :D]

    def sq(j):
        return swap_pieces(rq_ref, tq_ref, *FT[j])

    def sk(j):
        return swap_pieces(rk_ref, tk_ref, *FT[j])

    def mix(a, b):
        out = []
        for i, u in enumerate(a):
            out.append(u)
            out += b[(i * len(b)) // len(a):((i + 1) * len(b)) // len(a)]
        return out

    allh = range(H)
    lo3, all4 = [0, 1, 2], [0, 1, 2, 3]

    def vfull(heads):
        return mix(main_units(1, heads, 0, D, lo3), tt_units(1, heads, all4))

    v_cp[0].wait()
    swap(rv_ref, tv_ref, 0, 64)
    o_cp[0].wait()
    for i in range(6):
        v_cp[i + 1].wait()
        region(main_units(1, range(8), 64 * i, 64, lo3),
               swap_pieces(rv_ref, tv_ref, 64 * (i + 1), 64), skip=96)
    region(main_units(1, range(8), DM, 64, lo3) + tt_units(1, range(8), all4))
    o_cp[1].wait()
    for cp in small_cp:
        cp.wait()
    region(vfull(range(8, 12)), tt_pieces(1, range(4), all4) + col_pieces([6]))
    o_cp[2].wait()
    q_cp[0].wait()
    region(vfull(range(12, 14)), sq(0))
    k_cp[0].wait()
    region(vfull(range(14, 16)), sk(0))
    k_cp[1].wait()
    region(main_units(0, allh, 0, 128, [0]), sk(1), skip=64)
    q_cp[1].wait()
    region(main_units(0, allh, 128, 128, [0]), sq(1), skip=64)
    q_cp[3].wait()
    region(main_units(0, allh, 0, 256, [1]), mix(sq(3), tt_pieces(1, range(4, 8), all4)))
    k_cp[2].wait()
    region(tt_units(0, allh, [0, 1]), sk(2), skip=64)
    q_cp[2].wait()
    region(mix(main_units(0, allh, 256, 128, [0, 1]), tt_units(0, allh, [2])),
           mix(sq(2), tt_pieces(0, range(8), [0, 1])))
    k_cp[3].wait()
    x_cp[0].wait()
    mod_cp[0].wait()
    u = main_units(0, allh, 0, DM, [2])
    l0 = ln1_pieces(0)
    region(mix(u[:4], mod_units(0, MODA)) + u[4:],
           mix(sk(3), l0[:8]) + tt_pieces(0, range(8), [2]) + col_pieces([0, 1]))
    region(mix(main_units(0, allh, DM, 64, lo3), tt_units(0, allh, [3])),
           l0[8:] + ln1_pieces(1))
    mod_cp[1].wait()
    xl0 = x_lhs(0)
    jobs = ([(1, jc) for jc in chunks] + [(0, jc) for jc in chunks[2:] + chunks[:2]]
            + [(2, jc) for jc in gchunks])
    units = [(96, functools.partial(proj_chunk, xl0, kv, jc, xdst)) for kv, jc in jobs]
    wgp = ([functools.partial(wg_piece, hp, j) for hp in range(8) for j in range(3)]
           + tt_pieces(0, range(8), [3]))
    region(mix(units[:7], mod_units(MODA, 6 * D)) + units[7:26],
           wgp[:12] + mix(wgp[12:], col_pieces([2, 3, 4, 5])), skip=96)
    region(units[26:])
    x_cp[1].wait()
    for cp in mlp_cp:
        cp.start()

    def segment(k, hf, r0, sched, xl, ride, fill, tail=None):
        final = not isinstance(k, int)
        ks = 0 if final else k
        xs_ref, gs_ref = (xn_ref, gn_ref) if final else (xc_ref, gc_ref)
        hq = jnp.concatenate([hf, jnp.zeros((8, DX), F32)], axis=0).astype(BF16)
        lhs = hq[:32, :D]
        lhs_x = None if xl is None else jnp.concatenate([lhs, xl], axis=0)

        def nextp():
            pc = sched.pop(0) if sched else None
            return [] if pc is None else [pc]

        def chunk(kv, jc):
            if xl is not None and (kv, jc) in ride:
                proj_chunk(lhs_x, kv, jc, own + xdst, nextp())
            else:
                proj_chunk(lhs, kv, jc, own, nextp())

        def filler(n):
            for _ in range(n):
                if xl is not None and fill:
                    kv, jc = fill.pop(0)
                    proj_chunk(xl, kv, jc, xdst, nextp())

        parts = []
        for g in range(5):
            v = hf[8 * g:8 * g + 8, DM:]
            parts += [jnp.where(lo_half, v, 0.0), jnp.where(lo_half, 0.0, v)]
        b0 = jnp.concatenate(parts + [jnp.zeros((48, 128), F32)], axis=0).astype(BF16)

        for jc in gchunks:
            chunk(2, jc)
        for n_, jc in enumerate(chunks):
            chunk(0, jc)
            if n_ == 2:
                lg = _unpack(jnp.concatenate([g_ref[...], gs_ref[k]], axis=0))
                tt = jnp.concatenate(
                    [_dot_t(lg[80 * i:80 * i + 80], b0) for i in range(4)], axis=0)
                rr = [_roll(jnp.concatenate([tt[32 * hp:32 * hp + 32],
                                             tt[256 + 8 * hp:264 + 8 * hp]], axis=0), 16 * hp)
                      for hp in range(8)]
                s2 = [_roll(blocksel([rr[(b - g) % 8] for b in range(8)]), -16 * g)
                      for g in range(5)]
        lead = chunks[3 * ks:3 * ks + 3]
        vorder = lead + [jc for jc in chunks if jc not in lead]
        sc = {}
        chunk(1, vorder[0])
        for n_, g in enumerate((4, 0, 1, 2, 3)):
            kst = _unpack(xs_ref[0, k] if g == 4 else st_ref[0, g])
            sg = _dot_t(hq[:16 * QROWS[g]], kst)
            for q in range(5):
                if (q, g) not in VIS:
                    continue
                v = _r(sg[8 * q:8 * q + 8] + s2[g][8 * q:8 * q + 8])
                if q == g and g > 0:
                    v = jnp.where(tri, v, -1e9)
                sc[q, g] = v
            if n_ in (1, 3):
                chunk(1, vorder[(n_ + 1) // 2])
        per_q = [[g for g in range(5) if (q, g) in VIS] for q in range(5)]
        mx = jnp.concatenate([functools.reduce(jnp.maximum, [sc[q, g] for g in per_q[q]])
                              for q in range(5)], axis=0)
        mx = _group8_reduce(mx, jnp.maximum, lane40)
        ex = {qg: jnp.exp(v - mx[8 * qg[0]:8 * qg[0] + 8]) for qg, v in sc.items()}
        den = jnp.concatenate([functools.reduce(jnp.add, [ex[q, g] for g in per_q[q]])
                               for q in range(5)], axis=0)
        inv = 1.0 / _group8_reduce(den, jnp.add, lane40)
        zero8 = jnp.zeros((8, 128), F32)
        pg = [jnp.concatenate([ex[q, g] * inv[8 * q:8 * q + 8] if (q, g) in VIS else zero8
                               for q in range(5)], axis=0) for g in range(5)]
        pb = [jnp.concatenate([v, zero8], axis=0).astype(BF16) for v in pg]
        for jc in vorder[3:]:
            chunk(1, jc)
        filler(NFILL[0])
        outs = {}

        def out_main(j):
            cols = slice(128 * j, 128 * j + 128)
            v04 = jnp.concatenate([st_ref[1, 0, :, cols], xs_ref[1, k, :, cols]], axis=0)
            o3 = _dot(jnp.concatenate([pb[0], pb[4]], axis=1), _unpack(v04))
            v23 = jnp.concatenate([st_ref[1, 2, :, cols], st_ref[1, 3, :, cols]], axis=0)
            o2 = _dot(jnp.concatenate([pb[2][:32], pb[3][:32]], axis=1), _unpack(v23))
            o1 = _dot(pb[1][:16], _unpack(st_ref[1, 1, :, cols]))
            outs[j] = jnp.concatenate(
                [o3[:16] + o2[:16] + o1, o3[16:32] + o2[16:32], o3[32:40]], axis=0)

        for j in (3, 0, 1):
            out_main(j)
        filler(NFILL[1])
        pr = [_roll(pg[g], 16 * g) for g in range(5)]
        lz = jnp.concatenate(
            [_roll(blocksel([pr[(b - hp) % 8] if (b - hp) % 8 < 5 else None for b in range(8)]),
                   -16 * hp) for hp in range(8)], axis=0).astype(BF16)
        zt = [_dot(lz[80 * i:80 * i + 80], b0) for i in range(4)]
        zq = jnp.concatenate([zt[hp // 2][40 * (hp % 2):40 * (hp % 2) + 40]
                              for hp in range(8)], axis=1)
        if final:
            zq = jnp.concatenate([zq, jnp.zeros((8, 64 * H), F32)], axis=0).astype(BF16)
            nr = M + SEG
        else:
            zd_ref[k] = zq[32:]
            zq = zq[:32].astype(BF16)
            nr = 32
        out_main(2)
        filler(NFILL[2])
        for j in (3, 0, 1, 2):
            o2 = outs[j][:nr] + _dot(zq, _unpack(hr_ref[1, :, 128 * j:128 * j + 128]))[:nr]
            if not final:
                od_ref[k, 0:8, 128 * j:128 * j + 128] = outs[j][32:]
            outs[j] = o2
        hi = outs[3] + _roll(outs[3], DH)
        o = jnp.concatenate([outs[0], outs[1], outs[2], hi], axis=1)
        if final:
            a_ref[pl.ds(r0, 16), :] = _pack(jnp.concatenate([o[32:], o[16:32], o[8:16]], axis=0))
        else:
            od_ref[k, 8:16, :] = o[16:24]
            a_ref[pl.ds(r0 + 8, 8), :] = _pack(jnp.concatenate([o[24:32], o[8:16]], axis=0))
        if tail is not None:
            tail()
        filler(NFILL[3] if ks < 3 else NFILL[4])
        return _r(o[:M])

    def deferred(b):
        zq = zd_ref[...].reshape(32, 64 * H).astype(BF16)
        o2 = {j: _dot(zq, _unpack(hr_ref[1, :, 128 * j:128 * j + 128])) for j in (3, 0, 1, 2)}
        for k in range(4):
            t = [o2[j][8 * k:8 * k + 8] + od_ref[k, 0:8, 128 * j:128 * j + 128] for j in range(4)]
            t[3] = t[3] + _roll(t[3], DH)
            rows = jnp.concatenate([jnp.concatenate(t, axis=1), od_ref[k, 8:16, :]], axis=0)
            ra = b * (TB // 2) + k * (SEG // 2)
            if not isinstance(b, int):
                ra = pl.multiple_of(ra, SEG // 2)
            a_ref[pl.ds(ra, 8), :] = _pack(rows)

    def seg_rows(mem, r0):
        return jnp.concatenate([mem, h_ref[pl.ds(r0 + 24, 8), :], h_ref[pl.ds(r0 + 8, 16), :],
                                h_ref[pl.ds(r0, 8), :]], axis=0)

    def block(i, mem):
        prev = jnp.maximum(i - 1, 0)
        sched = []
        for u, v in zip(post_pieces(prev), ln1_pieces(jnp.minimum(i + 2, NB - 1))):
            sched += [None, None, None, v, None, None, None, u]
        xl = x_lhs(i + 1)
        xc_ref[...] = xn_ref[...]
        gc_ref[...] = gn_ref[...]
        nfill = 4 * sum(NFILL[:3]) + 3 * NFILL[3] + NFILL[4]
        alljobs = ([(0, jc) for jc in chunks] + [(1, jc) for jc in chunks[12:]]
                   + [(2, jc) for jc in gchunks])
        fill, rest = alljobs[:nfill], alljobs[nfill:]
        for k in range(4):
            ride = [(1, jc) for jc in chunks[3 * k:3 * k + 3]] + rest[k::4]
            r0 = pl.multiple_of(i * TB + k * SEG, SEG)
            ra = pl.multiple_of(i * (TB // 2) + k * (SEG // 2), SEG // 2)
            mem = segment(k, seg_rows(mem, r0), ra, sched, xl, ride, fill,
                          functools.partial(deferred, i) if k == 3 else None)
        assert not any(sched) and not fill
        return mem

    def last_segment(k, mem):
        r0 = pl.multiple_of((NB - 1) * TB + k * SEG, SEG)
        ra = pl.multiple_of((NB - 1) * (TB // 2) + k * (SEG // 2), SEG // 2)
        return segment(k, seg_rows(mem, r0), ra, [], None, (), [])

    m0 = mem0_ref[0].astype(F32)
    m0 = jnp.concatenate([m0, m0[:, DM:]], axis=1)
    mem = lax.fori_loop(0, NB - 1, block, m0)
    nfull = (NB - 2) * TB
    out_a = copy(ot_ref.at[:, pl.ds(0, nfull)], o_hbm.at[0, :, pl.ds(0, nfull)])
    out_a.start()
    lax.fori_loop(0, 4, last_segment, mem)

    for cp in mlp_cp:
        cp.wait()
    out_a.wait()
    for pa, pb in zip(post_pieces(NB - 2), post_pieces(NB - 1)):
        pa()
        pb()
    out_b = copy(ot_ref.at[:, pl.ds(nfull, 2 * TB)], o_hbm.at[0, :, pl.ds(nfull, 2 * TB)])
    out_b.start()

    bits = pltpu.bitcast(r_ref[...] + 0.0, jnp.int32)
    bits = jnp.where(bits < 0, bits ^ jnp.int32(0x7FFF0000), bits)
    tok = (lax.broadcasted_iota(jnp.int32, (NB, TB), 0) * TB
           + lax.broadcasted_iota(jnp.int32, (NB, TB), 1))
    idx = (S - 1) - (jnp.max(bits | ((S - 1) - tok)) & (S - 1))
    blk = idx // TB
    ln = idx - blk * TB
    t0 = pl.multiple_of(blk * TB, TB)
    h2 = _unpack(h2_ref[:, pl.ds(t0, TB)])
    onehot = (lax.broadcasted_iota(jnp.int32, (8, TB), 1) == ln)
    hsel = _dot_t(onehot.astype(BF16), h2).astype(BF16)
    gt = _r(_dot(hsel, wg_ref[...]))
    gt = _r(gt * jax.nn.sigmoid(gt))
    up = _r(_dot(hsel, wu_ref[...]))
    y = _r(_dot_t(_r(gt * up).astype(BF16), wdt_ref[...]))
    yt = jnp.broadcast_to(y[0:1], (TB, D)).T
    yt = _r(yt * _r(jax.nn.sigmoid(r_ref[pl.ds(blk, 1), :])))
    h2 = h2.astype(F32)
    sel = lax.broadcasted_iota(jnp.int32, (D, TB), 1) == ln
    hb2 = jnp.where(sel, _r(h2 + yt), h2)
    fix = (x1_ref[:, pl.ds(t0, TB)] + col_ref[5] * hb2).astype(BF16)
    out_b.wait()
    ot_ref[:, pl.ds(t0, TB)] = fix
    out_c = copy(ot_ref.at[:, pl.ds(t0, TB)], o_hbm.at[0, :, pl.ds(t0, TB)])
    out_c.start()
    out_c.wait()


@jax.jit
def pallas_adaLN_cond__memory_aug_recurrent_mem_tr__moe_arch_mod__prompt_kernel(
        A_x, A_mem0, A_Wq, A_Wk, A_Wv, A_Wo, A_seg_len, B_x, B_w_r, B_w_gate, B_w_up,
        B_w_down, c, w_mod):
    del A_seg_len, B_x
    any_spec = pl.BlockSpec(memory_space=pl.ANY)
    out_t = pl.pallas_call(
        _kernel,
        out_shape=jax.ShapeDtypeStruct((1, D, S), BF16),
        in_specs=[any_spec] * 12,
        out_specs=any_spec,
        scratch_shapes=[
            pltpu.VMEM((1, M, D), BF16),
            pltpu.VMEM((D,), BF16),
            pltpu.VMEM((1, D), BF16),
            pltpu.VMEM((D, S), BF16),
            pltpu.VMEM((D, H, E), BF16),
            pltpu.VMEM((D, H, E), BF16),
            pltpu.VMEM((D, H, E), BF16),
            pltpu.VMEM((H, D, E), BF16),
            pltpu.VMEM((D, FF), BF16),
            pltpu.VMEM((D, FF), BF16),
            pltpu.VMEM((D, FF), BF16),
            pltpu.VMEM((D, 6 * D), BF16),
            pltpu.VMEM((D, S), BF16),
            pltpu.VMEM((S, DX), F32),
            pltpu.VMEM((S // 2, DX), U32),
            pltpu.VMEM((H, D // 2, E), U32),
            pltpu.VMEM((H, D // 2, E), U32),
            pltpu.VMEM((H, D // 2, E), U32),
            pltpu.VMEM((DM // 2, NT * 128), U32),
            pltpu.VMEM((DM // 2, NT * 128), U32),
            pltpu.VMEM((2, 4, 64, DX), U32),
            pltpu.VMEM((2, 4, 64, DX), U32),
            pltpu.VMEM((2, 4, 64, DX), U32),
            pltpu.VMEM((2, 32 * H, DX), U32),
            pltpu.VMEM((2, 32 * H, DX), U32),
            pltpu.VMEM((D // 2, 64 * H), U32),
            pltpu.VMEM((128, 128), U32),
            pltpu.VMEM((4, 32, 128), U32),
            pltpu.VMEM((4, 32, 128), U32),
            pltpu.VMEM((4, 8, 64 * H), F32),
            pltpu.VMEM((4, 16, DX), F32),
            pltpu.VMEM((8, 6 * D), F32),
            pltpu.VMEM((7, D, TB), F32),
            pltpu.VMEM((NB, TB), F32),
            pltpu.VMEM((D, S), F32),
            pltpu.VMEM((D // 2, S), U32),
            pltpu.VMEM((8, 128), U32),
            pltpu.SemaphoreType.DMA((32,)),
        ],
        compiler_params=pltpu.CompilerParams(vmem_limit_bytes=120 * 1024 * 1024),
    )(jnp.swapaxes(A_x, 1, 2), A_mem0, A_Wq, A_Wk, A_Wv, jnp.swapaxes(A_Wo, 1, 2),
      B_w_r, B_w_gate, B_w_up, B_w_down.T, c, w_mod)
    return jnp.swapaxes(out_t, 1, 2)
```
